```python
import os as _os
_os.environ.setdefault("JAX_PLATFORMS", "cpu")
import jax
import jax.numpy as jnp

def _softmax(x, axis=-1):
    return jax.nn.softmax(x, axis=axis)
def _gelu(x):
    return jax.nn.gelu(x, approximate=True)
def _silu(x):
    return jax.nn.silu(x)
def _sigmoid(x):
    return jax.nn.sigmoid(x)
def _layernorm(x, axis=-1, eps=1e-5):
    m = jnp.mean(x, axis=axis, keepdims=True)
    v = jnp.var(x, axis=axis, keepdims=True)
    return (x - m) / jnp.sqrt(v + eps)
def _scatter_add(tgt, idx, src, axis=0):
    return tgt.at[idx].add(src)
def _segment_sum(src, seg, n):
    return jax.ops.segment_sum(src, seg, n)
class _Rng:
    def __init__(self, key):
        self._k = key
    def _next(self):
        self._k, sub = jax.random.split(self._k)
        return sub
    def normal(self, shape):
        return jax.random.normal(self._next(), shape, dtype=jnp.bfloat16)
    def randint(self, lo, hi, shape):
        return jax.random.randint(self._next(), shape, lo, hi, dtype=jnp.int32)
    def uniform(self, shape, lo=0.0, hi=1.0):
        return jax.random.uniform(self._next(), shape, jnp.bfloat16, lo, hi)
    def permutation(self, n):
        return jax.random.permutation(self._next(), n)


kernel_name = 'gated_mix__sliding_block_cached__swiglu_ffn__decode'

def setup_inputs():
    _rng = _Rng(jax.random.key(int.from_bytes(__import__("os").urandom(4), "little")))
    _w = (lambda a: (lambda t: t.astype(jnp.bfloat16) if jnp.issubdtype(t.dtype, jnp.floating) else t)(jnp.asarray(a)))
    def _A_setup():
        B, Sq, D = 1, 1, 512
        Hq, Hkv, Sk, Dh = 32, 32, 32768, 128
        assert Hq % Hkv == 0, (Hq, Hkv)
        return {
            "x": _w((lambda *s: _rng.normal(s) * 0.05)(B, Sq, D)),
            "k_cache": _w((lambda *s: _rng.normal(s) * 3.2)(B, Hkv, Sk, Dh)),
            "v_cache": _w((lambda *s: _rng.normal(s) * 1.6)(B, Hkv, Sk, Dh)),
            "wq": _w((lambda *s: _rng.normal(s) * 3.2)(D, Hq * Dh) * (D ** -0.5)),
            "wo": _w((lambda *s: _rng.normal(s) * 1.6)(Hq * Dh, D) * ((Hq * Dh) ** -0.5)),
        }
    _A_in = _A_setup()

    def _B_setup():
        B, S, D, F = 1, 1, 512, 1376
        return {
            "x": _w((lambda *s: _rng.normal(s) * 0.05)(B, S, D)),
            "w_gate": _w((lambda *s: _rng.normal(s) * 0.1)(D, F)),
            "w_up": _w((lambda *s: _rng.normal(s) * 0.1)(D, F)),
            "w_down": _w((lambda *s: _rng.normal(s) * 0.1)(F, D)),
        }
    _B_in = _B_setup()

    return {
        "A_x": _A_in["x"],
        "A_k_cache": _A_in["k_cache"],
        "A_v_cache": _A_in["v_cache"],
        "A_wq": _A_in["wq"],
        "A_wo": _A_in["wo"],
        "B_x": _B_in["x"],
        "B_w_gate": _B_in["w_gate"],
        "B_w_up": _B_in["w_up"],
        "B_w_down": _B_in["w_down"],
        "gate_w": _w((lambda *s: _rng.normal(s) * 0.05)(512) * 16.0),
    }

def reference(A_x, A_k_cache, A_v_cache, A_wq, A_wo, B_x, B_w_gate, B_w_up, B_w_down, gate_w):
    def _A_ref(x, k_cache, v_cache, wq, wo):
        B, Sq, D = x.shape
        Hq, Dh = 32, 128
        Hkv, Sk = k_cache.shape[1], k_cache.shape[2]
        W = min(4096, max(256, Sk // 4))
        rep = Hq // Hkv
        q = (lambda x, *d: x.transpose(*d))((x @ wq).reshape(B, Sq, Hq, Dh), 0, 2, 1, 3)
        k = jnp.repeat(k_cache[:, :, Sk - W:, :], rep, axis=1)
        v = jnp.repeat(v_cache[:, :, Sk - W:, :], rep, axis=1)
        scores = jnp.einsum("bhqd,bhkd->bhqk", q, k) * (Dh ** -0.5)
        p = _softmax(scores, axis=-1)
        o = jnp.einsum("bhqk,bhkd->bhqd", p, v)
        return (lambda x, *d: x.transpose(*d))(o, 0, 2, 1, 3).reshape(B, Sq, Hq * Dh) @ wo

    def _B_ref(x, w_gate, w_up, w_down):
        g = _silu(x @ w_gate)
        u = x @ w_up
        return (g * u) @ w_down

    x = A_x
    g = _sigmoid((x * gate_w).sum(-1, keepdims=True))
    a = _A_ref(x, A_k_cache, A_v_cache, A_wq, A_wo)
    b = _B_ref(x, B_w_gate, B_w_up, B_w_down)
    return g * a + (1 - g) * b
```

```python
import jax
import jax.numpy as jnp
from jax import lax
import jax.experimental.pallas as pl
import jax.experimental.pallas.tpu as pltpu

HQ, DH = 32, 128
M = 8
NB = 2
NT = (((1,), (1,)), ((), ()))


@jax.jit
def pallas_gated_mix__sliding_block_cached__swiglu_ffn__decode_kernel(
    A_x: jax.Array,
    A_k_cache: jax.Array,
    A_v_cache: jax.Array,
    A_wq: jax.Array,
    A_wo: jax.Array,
    B_x: jax.Array,
    B_w_gate: jax.Array,
    B_w_up: jax.Array,
    B_w_down: jax.Array,
    gate_w: jax.Array,
):
    D = A_x.shape[-1]
    Sk = A_k_cache.shape[2]
    W = min(4096, max(256, Sk // 4))
    F = B_w_down.shape[0]
    bf = jnp.bfloat16
    f32 = jnp.float32
    scale = DH ** -0.5
    nb = NB

    def kernel(x_hbm, k_hbm, v_hbm, wq_hbm, wo_hbm, wg_hbm, wu_hbm, wd_hbm, gw_hbm, o_ref,
               xb, gwb, wqb, wob, wgb, wub, wdb, kb, vb, ksem, vsem, wsem):
      def kcp(h, slot):
        return pltpu.make_async_copy(k_hbm.at[0, h, pl.ds(Sk - W, W), :], kb.at[slot], ksem.at[slot])
      def vcp(h, slot):
        return pltpu.make_async_copy(v_hbm.at[0, h, pl.ds(Sk - W, W), :], vb.at[slot], vsem.at[slot])
      c_wq = pltpu.make_async_copy(wq_hbm, wqb, wsem.at[0])
      c_x = pltpu.make_async_copy(x_hbm, xb, wsem.at[1])
      c_gw = pltpu.make_async_copy(gw_hbm, gwb, wsem.at[2])
      c_wo = pltpu.make_async_copy(wo_hbm, wob, wsem.at[3])
      c_wg = pltpu.make_async_copy(wg_hbm, wgb, wsem.at[4])
      c_wu = pltpu.make_async_copy(wu_hbm, wub, wsem.at[5])
      c_wd = pltpu.make_async_copy(wd_hbm, wdb, wsem.at[6])
      c_wq.start()
      c_x.start()
      c_gw.start()
      c_wo.start()
      c_wg.start()
      c_wu.start()
      for s in range(nb):
        kcp(s, s).start()
        vcp(s, s).start()
      c_x.wait()
      c_gw.wait()
      x1 = xb[0].astype(f32)
      xm = jnp.broadcast_to(x1, (M, D)).astype(bf)
      gw = gwb[...].astype(f32)
      z = sum(x1[:, j * 128:(j + 1) * 128] * gw[j:j + 1, :] for j in range(D // 128))
      gate = jax.nn.sigmoid(jnp.sum(z, axis=-1, keepdims=True))
      c_wq.wait()
      c_wo.wait()
      c_wg.wait()
      c_wu.wait()
      g = lax.dot_general(xm, wgb[...], NT, preferred_element_type=f32)
      u = lax.dot_general(xm, wub[...], NT, preferred_element_type=f32)
      hid = (g * jax.nn.sigmoid(g) * u).astype(bf)

      def head(h, acc):
        slot = h % nb
        col = pl.ds(pl.multiple_of(h * DH, DH), DH)
        q = jnp.dot(xm, wqb[:, col], preferred_element_type=f32).astype(bf)
        kcp(h, slot).wait()
        s = lax.dot_general(q, kb[slot], NT, preferred_element_type=f32) * scale
        m = jnp.max(s, axis=-1, keepdims=True)
        p = jnp.exp(s - m)
        l = jnp.sum(p, axis=-1, keepdims=True)
        pb = p.astype(bf)

        @pl.when(h + nb < HQ)
        def _():
          kcp(h + nb, slot).start()

        @pl.when(h + nb == HQ)
        def _():
          c_wd.start()
        vcp(h, slot).wait()
        o = jnp.dot(pb, vb[slot], preferred_element_type=f32) / l

        @pl.when(h + nb < HQ)
        def _():
          vcp(h + nb, slot).start()
        return acc + jnp.dot(o.astype(bf), wob[col, :], preferred_element_type=f32)

      a = lax.fori_loop(0, HQ, head, jnp.zeros((M, D), f32))
      c_wd.wait()
      b = jnp.dot(hid, wdb[...], preferred_element_type=f32)
      out = gate * a[0:1] + (1.0 - gate) * b[0:1]
      o_ref[0] = out.astype(o_ref.dtype)

    hbm = pl.BlockSpec(memory_space=pltpu.HBM)
    return pl.pallas_call(
        kernel,
        out_shape=jax.ShapeDtypeStruct(A_x.shape, A_x.dtype),
        in_specs=[hbm] * 9,
        out_specs=pl.BlockSpec(memory_space=pltpu.VMEM),
        scratch_shapes=[
            pltpu.VMEM(A_x.shape, bf), pltpu.VMEM((D // 128, 128), bf),
            pltpu.VMEM(A_wq.shape, bf), pltpu.VMEM(A_wo.shape, bf),
            pltpu.VMEM((F, D), bf), pltpu.VMEM((F, D), bf), pltpu.VMEM((F, D), bf),
            pltpu.VMEM((nb, W, DH), bf), pltpu.VMEM((nb, W, DH), bf),
            pltpu.SemaphoreType.DMA((nb,)), pltpu.SemaphoreType.DMA((nb,)), pltpu.SemaphoreType.DMA((7,)),
        ],
        compiler_params=pltpu.CompilerParams(vmem_limit_bytes=100 * 1024 * 1024),
    )(A_x, A_k_cache, A_v_cache, A_wq, A_wo, B_w_gate.T, B_w_up.T, B_w_down, gate_w.reshape(D // 128, 128))
```

```python
import functools

import jax
import jax.numpy as jnp
import numpy as np
from jax import lax
import jax.experimental.pallas as pl
import jax.experimental.pallas.tpu as pltpu

_HQ, _DH = 32, 128
_HG = 8
_CHUNK = 512
_PIECE = 64
_PAIRS = _HG // 2
_NSEM = 3
_LAST_STAGE = 96
_NT = (((1,), (1,)), ((), ()))
_F32_MIN = float(np.finfo(np.float32).min)


def _loop(n, body):
    def step(j, carry):
        body(j)
        return carry

    lax.fori_loop(0, n, step, 0)


def _wait_filled(buf, sem):
    pltpu.make_async_copy(buf, buf, sem).wait()


def _row_h_of(vals):
    row = lax.broadcasted_iota(jnp.int32, vals[0].shape, 0)
    out = vals[0]
    for h in range(1, len(vals)):
        out = jnp.where(row == h, vals[h], out)
    return out


def _kernel(x_hbm, k_hbm, v_hbm, wq_hbm, wo_hbm, wg_hbm, wu_hbm, wd_hbm, gw_hbm,
            o_ref,
            x_buf, gw_buf, wq_buf, wo_buf, wg_buf, wu_buf, wd_buf, k_buf, v_buf, sems,
            *, window):
    f32 = jnp.float32
    mxu_dtype = k_buf.dtype
    ffn, d_model = wd_buf.shape
    win_start = k_hbm.shape[2] - window
    n_chunks = window // _CHUNK
    n_groups = _HQ // _HG
    n_steps = n_groups * n_chunks
    n_pieces = _CHUNK // _PIECE
    wd_rows = 2 * _PIECE * _DH // d_model
    wd_first = n_pieces * _PAIRS * wd_rows
    wd_stages = (wd_first, ffn - wd_first - _LAST_STAGE, _LAST_STAGE)

    def sem_of(step):
        return sems.at[lax.rem(step, _NSEM)]

    def cache_copy(src, dst, step, j, t):
        head = lax.div(step, n_chunks) * _HG + 2 * t
        row = pl.multiple_of(j * _PIECE, _PIECE)
        src_row = pl.multiple_of(win_start + lax.rem(step, n_chunks) * _CHUNK + row, _PIECE)
        return pltpu.make_async_copy(
            src.at[0, pl.ds(head, 2), pl.ds(src_row, _PIECE), :],
            dst.at[lax.rem(step, dst.shape[0]), pl.ds(2 * t, 2), pl.ds(row, _PIECE), :],
            sem_of(step))

    k_copy = functools.partial(cache_copy, k_hbm, k_buf)
    v_copy = functools.partial(cache_copy, v_hbm, v_buf)

    def wd_copy(step, j, t):
        rows = pl.ds(pl.multiple_of((j * _PAIRS + t) * wd_rows, wd_rows), wd_rows)
        return pltpu.make_async_copy(wd_hbm.at[rows, :], wd_buf.at[rows, :], sem_of(step))

    def wd_stage(i):
        rows = pl.ds(sum(wd_stages[:i]), wd_stages[i])
        return pltpu.make_async_copy(
            wd_hbm.at[rows, :], wd_buf.at[rows, :], sems.at[(n_steps + i) % _NSEM])

    def start_step(step, ahead_copy):
        def body(j):
            for t in range(_PAIRS):
                k_copy(step, j, t).start(priority=0)
                ahead_copy(step + 1, j, t).start(priority=1)

        _loop(n_pieces, body)

    ffn_sem, proj_sem = sems.at[1], sems.at[2]

    def start_gate_up(j):
        rows = pl.ds(pl.multiple_of(j * 16, 16), 16)
        pltpu.make_async_copy(wg_hbm.at[:, rows, :], wg_buf.at[:, rows, :], ffn_sem).start(priority=0)
        pltpu.make_async_copy(wu_hbm.at[:, rows, :], wu_buf.at[:, rows, :], ffn_sem).start(priority=1)

    _loop(wg_buf.shape[1] // 16, start_gate_up)
    x_copy = pltpu.make_async_copy(x_hbm, x_buf, ffn_sem)
    gw_copy = pltpu.make_async_copy(gw_hbm, gw_buf, ffn_sem)
    x_copy.start()
    gw_copy.start()

    wq_cols = 2 * d_model
    wq_col_blocks = _HQ * _DH // wq_cols

    def start_projections(j):
        q_rows = pl.ds(pl.multiple_of(lax.div(j, wq_col_blocks) * 8, 8), 8)
        q_cols = pl.ds(pl.multiple_of(lax.rem(j, wq_col_blocks) * wq_cols, wq_cols), wq_cols)
        o_rows = pl.ds(pl.multiple_of(j * 16, 16), 16)
        for t in range(wq_buf.shape[0]):
            pltpu.make_async_copy(wq_hbm.at[t, :, q_rows, q_cols], wq_buf.at[t, :, q_rows, q_cols],
                                  proj_sem).start(priority=0)
            pltpu.make_async_copy(wo_hbm.at[t, :, o_rows, :], wo_buf.at[t, :, o_rows, :],
                                  proj_sem).start(priority=1)

    _loop(wo_buf.shape[2] // 16, start_projections)

    x_copy.wait()
    gw_copy.wait()
    _wait_filled(wg_buf, ffn_sem)
    _wait_filled(wu_buf, ffn_sem)
    x = x_buf[0].astype(f32)
    x_rows = jnp.broadcast_to(x, (_HG, d_model)).astype(mxu_dtype)
    gate_w = gw_buf[...].astype(f32)
    lanes = gate_w.shape[1]
    logit = sum(x[:, i * lanes:(i + 1) * lanes] * gate_w[i:i + 1, :] for i in range(gate_w.shape[0]))
    gate = jax.nn.sigmoid(jnp.sum(logit, axis=-1, keepdims=True))
    pre_gate = lax.dot_general(x_rows, wg_buf[...].reshape(ffn, d_model), _NT, preferred_element_type=f32)
    pre_up = lax.dot_general(x_rows, wu_buf[...].reshape(ffn, d_model), _NT, preferred_element_type=f32)
    hidden = (pre_gate * jax.nn.sigmoid(pre_gate) * pre_up).astype(mxu_dtype)

    def start_first_v(j):
        for t in range(_PAIRS):
            v_copy(0, j, t).start(priority=t % 2)

    _loop(n_pieces, start_first_v)
    start_step(0, v_copy)
    _wait_filled(wq_buf, proj_sem)
    _wait_filled(wo_buf, proj_sem)

    def group(g, acc):
        cols = pl.ds(pl.multiple_of(g * (_HG * _DH), _HG * _DH), _HG * _DH)
        q_all = jnp.dot(x_rows, wq_buf[:, :, :, cols].reshape(d_model, _HG * _DH), preferred_element_type=f32)
        q = _row_h_of([q_all[:, h * _DH:(h + 1) * _DH] for h in range(_HG)]).astype(mxu_dtype)

        def chunk(c, carry):
            m, l, o = carry
            step = g * n_chunks + c

            @pl.when(step + 2 < n_steps)
            def _():
                start_step(step + 1, v_copy)

            @pl.when(step + 2 == n_steps)
            def _():
                start_step(step + 1, wd_copy)

            k_slot = lax.rem(step, k_buf.shape[0])
            v_slot = lax.rem(step, v_buf.shape[0])
            _wait_filled(k_buf.at[k_slot], sem_of(step))
            _wait_filled(v_buf.at[v_slot], sem_of(step))

            @pl.when(step + 1 == n_steps)
            def _():
                for i in range(1, len(wd_stages)):
                    wd_stage(i).start(priority=1)

            s = _row_h_of([lax.dot_general(q, k_buf[k_slot, h], _NT, preferred_element_type=f32)
                           for h in range(_HG)]) * (_DH ** -0.5)
            m_new = jnp.maximum(m, jnp.max(s, axis=-1, keepdims=True))
            alpha = jnp.exp(m - m_new)
            p = jnp.exp(s - m_new)
            l_new = alpha * l + jnp.sum(p, axis=-1, keepdims=True)
            p = p.astype(mxu_dtype)
            pv = _row_h_of([jnp.dot(p, v_buf[v_slot, h], preferred_element_type=f32) for h in range(_HG)])
            return m_new, l_new, alpha * o + pv

        init = (jnp.full((_HG, 1), _F32_MIN, f32), jnp.zeros((_HG, 1), f32), jnp.zeros((_HG, _DH), f32))
        _, l, o = lax.fori_loop(0, n_chunks, chunk, init)
        o = (o / l).astype(mxu_dtype)
        per_half = _HG // 2
        return acc + _row_h_of([
            jnp.dot(o, wo_buf[g, h // per_half, pl.ds((h % per_half) * _DH, _DH), :], preferred_element_type=f32)
            for h in range(_HG)])

    attn = lax.fori_loop(0, n_groups, group, jnp.zeros((_HG, d_model), f32))

    out = gate * jnp.sum(attn, axis=0, keepdims=True)
    lo = 0
    for i, rows in enumerate(wd_stages):
        wd_stage(i).wait()
        part = jnp.dot(hidden[:, lo:lo + rows], wd_buf[lo:lo + rows, :], preferred_element_type=f32)
        out = out + (1.0 - gate) * part[0:1]
        lo += rows
    o_ref[0] = out.astype(o_ref.dtype)


@jax.jit
def pallas_gated_mix__sliding_block_cached__swiglu_ffn__decode_kernel(
    A_x: jax.Array,
    A_k_cache: jax.Array,
    A_v_cache: jax.Array,
    A_wq: jax.Array,
    A_wo: jax.Array,
    B_x: jax.Array,
    B_w_gate: jax.Array,
    B_w_up: jax.Array,
    B_w_down: jax.Array,
    gate_w: jax.Array,
):
    del B_x
    d_model = A_x.shape[-1]
    ffn = B_w_down.shape[0]
    cache_len = A_k_cache.shape[2]
    window = min(4096, max(256, cache_len // 4))
    assert A_x.shape == (1, 1, d_model) and A_k_cache.shape == (1, _HQ, cache_len, _DH)
    assert window % _CHUNK == 0 and cache_len % _PIECE == 0 and ffn % 32 == 0

    wq = A_wq.reshape(_HQ // _HG, 2, d_model // 8, _HQ * _DH)
    wo = A_wo.reshape(_HQ // _HG, 2, _HG * _DH // 2, d_model)
    wg = B_w_gate.T.reshape(2, ffn // 2, d_model)
    wu = B_w_up.T.reshape(2, ffn // 2, d_model)
    gw = gate_w.reshape(d_model // 128, 128)
    operands = (A_x, A_k_cache, A_v_cache, wq, wo, wg, wu, B_w_down, gw)

    return pl.pallas_call(
        functools.partial(_kernel, window=window),
        out_shape=jax.ShapeDtypeStruct(A_x.shape, A_x.dtype),
        in_specs=[pl.BlockSpec(memory_space=pltpu.HBM)] * len(operands),
        out_specs=pl.BlockSpec(memory_space=pltpu.VMEM),
        scratch_shapes=[
            *(pltpu.VMEM(a.shape, a.dtype) for a in (A_x, gw, wq, wo, wg, wu, B_w_down)),
            pltpu.VMEM((2, _HG, _CHUNK, _DH), A_k_cache.dtype),
            pltpu.VMEM((_NSEM, _HG, _CHUNK, _DH), A_v_cache.dtype),
            pltpu.SemaphoreType.DMA((_NSEM,)),
        ],
        compiler_params=pltpu.CompilerParams(vmem_limit_bytes=48 * 1024 * 1024),
    )(*operands)
```

```python
import functools

import jax
import jax.numpy as jnp
import numpy as np
from jax import lax
import jax.experimental.pallas as pl
import jax.experimental.pallas.tpu as pltpu

_HQ, _DH = 32, 128
_HG = 8
_CHUNK = 512
_PIECE = 64
_PAIRS = _HG // 2
_NSEM = 3
_LAST_STAGE = 96
_NT = (((1,), (1,)), ((), ()))
_F32_MIN = float(np.finfo(np.float32).min)


def _loop(n, body):
    def step(j, carry):
        body(j)
        return carry

    lax.fori_loop(0, n, step, 0)


def _wait_filled(buf, sem):
    pltpu.make_async_copy(buf, buf, sem).wait()


def _row_h_of(vals):
    row = lax.broadcasted_iota(jnp.int32, vals[0].shape, 0)
    out = vals[0]
    for h in range(1, len(vals)):
        out = jnp.where(row == h, vals[h], out)
    return out


def _kernel(x_hbm, k_hbm, v_hbm, wq_hbm, wo_hbm, wg_hbm, wu_hbm, wd_hbm, gw_hbm,
            o_ref,
            x_buf, gw_buf, wq_buf, wo_buf, wg_buf, wu_buf, wd_buf, k_buf, v_buf, sems,
            *, window):
    f32 = jnp.float32
    mxu_dtype = k_buf.dtype
    ffn, d_model = wd_buf.shape
    win_start = k_hbm.shape[2] - window
    n_chunks = window // _CHUNK
    n_groups = _HQ // _HG
    n_steps = n_groups * n_chunks
    n_pieces = _CHUNK // _PIECE
    wd_rows = 2 * _PIECE * _DH // d_model
    wd_first = n_pieces * _PAIRS * wd_rows
    wd_stages = (wd_first, ffn - wd_first - _LAST_STAGE, _LAST_STAGE)

    def sem_of(step):
        return sems.at[lax.rem(step, _NSEM)]

    def cache_copy(src, dst, step, j, t):
        head = lax.div(step, n_chunks) * _HG + 2 * t
        row = pl.multiple_of(j * _PIECE, _PIECE)
        src_row = pl.multiple_of(win_start + lax.rem(step, n_chunks) * _CHUNK + row, _PIECE)
        return pltpu.make_async_copy(
            src.at[0, pl.ds(head, 2), pl.ds(src_row, _PIECE), :],
            dst.at[lax.rem(step, dst.shape[0]), pl.ds(2 * t, 2), pl.ds(row, _PIECE), :],
            sem_of(step))

    k_copy = functools.partial(cache_copy, k_hbm, k_buf)
    v_copy = functools.partial(cache_copy, v_hbm, v_buf)

    def wd_copy(step, j, t):
        rows = pl.ds(pl.multiple_of((j * _PAIRS + t) * wd_rows, wd_rows), wd_rows)
        return pltpu.make_async_copy(wd_hbm.at[rows, :], wd_buf.at[rows, :], sem_of(step))

    def wd_stage(i):
        return pl.ds(sum(wd_stages[:i]), wd_stages[i]), sems.at[(n_steps + i) % _NSEM]

    def start_step(step, ahead_copy):
        def body(j):
            for t in range(_PAIRS):
                k_copy(step, j, t).start(priority=0)
                ahead_copy(step + 1, j, t).start(priority=1)

        _loop(n_pieces, body)

    ffn_sem, proj_sem = sems.at[1], sems.at[2]

    def start_gate_up(j):
        rows = pl.ds(pl.multiple_of(j * 16, 16), 16)
        pltpu.make_async_copy(wg_hbm.at[:, rows, :], wg_buf.at[:, rows, :], ffn_sem).start(priority=0)
        pltpu.make_async_copy(wu_hbm.at[:, rows, :], wu_buf.at[:, rows, :], ffn_sem).start(priority=1)

    _loop(wg_buf.shape[1] // 16, start_gate_up)
    x_copy = pltpu.make_async_copy(x_hbm, x_buf, ffn_sem)
    gw_copy = pltpu.make_async_copy(gw_hbm, gw_buf, ffn_sem)
    x_copy.start()
    gw_copy.start()

    wq_cols = 2 * d_model
    wq_col_blocks = _HQ * _DH // wq_cols

    def start_projections(j):
        q_rows = pl.ds(pl.multiple_of(lax.div(j, wq_col_blocks) * 8, 8), 8)
        q_cols = pl.ds(pl.multiple_of(lax.rem(j, wq_col_blocks) * wq_cols, wq_cols), wq_cols)
        o_rows = pl.ds(pl.multiple_of(j * 16, 16), 16)
        for t in range(wq_buf.shape[0]):
            pltpu.make_async_copy(wq_hbm.at[t, :, q_rows, q_cols], wq_buf.at[t, :, q_rows, q_cols],
                                  proj_sem).start(priority=0)
            pltpu.make_async_copy(wo_hbm.at[t, :, o_rows, :], wo_buf.at[t, :, o_rows, :],
                                  proj_sem).start(priority=1)

    _loop(wo_buf.shape[2] // 16, start_projections)

    x_copy.wait()
    gw_copy.wait()
    _wait_filled(wg_buf, ffn_sem)
    _wait_filled(wu_buf, ffn_sem)
    x = x_buf[0].astype(f32)
    x_rows = jnp.broadcast_to(x, (_HG, d_model)).astype(mxu_dtype)
    gate_w = gw_buf[...].astype(f32)
    lanes = gate_w.shape[1]
    logit = sum(x[:, i * lanes:(i + 1) * lanes] * gate_w[i:i + 1, :] for i in range(gate_w.shape[0]))
    gate = jax.nn.sigmoid(jnp.sum(logit, axis=-1, keepdims=True))
    pre_gate = lax.dot_general(x_rows, wg_buf[...].reshape(ffn, d_model), _NT, preferred_element_type=f32)
    pre_up = lax.dot_general(x_rows, wu_buf[...].reshape(ffn, d_model), _NT, preferred_element_type=f32)
    hidden = (pre_gate * jax.nn.sigmoid(pre_gate) * pre_up).astype(mxu_dtype)

    def start_first_v(j):
        for t in range(_PAIRS):
            v_copy(0, j, t).start(priority=t % 2)

    _loop(n_pieces, start_first_v)
    start_step(0, v_copy)
    _wait_filled(wq_buf, proj_sem)
    _wait_filled(wo_buf, proj_sem)

    def group(g, acc):
        cols = pl.ds(pl.multiple_of(g * (_HG * _DH), _HG * _DH), _HG * _DH)
        q_all = jnp.dot(x_rows, wq_buf[:, :, :, cols].reshape(d_model, _HG * _DH), preferred_element_type=f32)
        q = _row_h_of([q_all[:, h * _DH:(h + 1) * _DH] for h in range(_HG)]).astype(mxu_dtype)

        def chunk(c, carry):
            m, l, o = carry
            step = g * n_chunks + c

            @pl.when(step + 2 < n_steps)
            def _():
                start_step(step + 1, v_copy)

            @pl.when(step + 2 == n_steps)
            def _():
                start_step(step + 1, wd_copy)

            k_slot = lax.rem(step, k_buf.shape[0])
            v_slot = lax.rem(step, v_buf.shape[0])
            _wait_filled(k_buf.at[k_slot], sem_of(step))
            _wait_filled(v_buf.at[v_slot], sem_of(step))

            @pl.when(step + 1 == n_steps)
            def _():
                for i in range(1, len(wd_stages)):
                    rows, sem = wd_stage(i)
                    pltpu.make_async_copy(wd_hbm.at[rows, :], wd_buf.at[rows, :], sem).start(priority=1)

            s = _row_h_of([lax.dot_general(q, k_buf[k_slot, h], _NT, preferred_element_type=f32)
                           for h in range(_HG)]) * (_DH ** -0.5)
            m_new = jnp.maximum(m, jnp.max(s, axis=-1, keepdims=True))
            alpha = jnp.exp(m - m_new)
            p = jnp.exp(s - m_new)
            l_new = alpha * l + jnp.sum(p, axis=-1, keepdims=True)
            p = p.astype(mxu_dtype)
            pv = _row_h_of([jnp.dot(p, v_buf[v_slot, h], preferred_element_type=f32) for h in range(_HG)])
            return m_new, l_new, alpha * o + pv

        init = (jnp.full((_HG, 1), _F32_MIN, f32), jnp.zeros((_HG, 1), f32), jnp.zeros((_HG, _DH), f32))
        _, l, o = lax.fori_loop(0, n_chunks, chunk, init)
        o = (o / l).astype(mxu_dtype)
        per_half = _HG // 2
        return acc + _row_h_of([
            jnp.dot(o, wo_buf[g, h // per_half, pl.ds((h % per_half) * _DH, _DH), :], preferred_element_type=f32)
            for h in range(_HG)])

    attn = lax.fori_loop(0, n_groups, group, jnp.zeros((_HG, d_model), f32))

    out = gate * jnp.sum(attn, axis=0, keepdims=True)
    for i in range(len(wd_stages)):
        rows, sem = wd_stage(i)
        _wait_filled(wd_buf.at[rows, :], sem)
        part = jnp.dot(hidden[:, rows.start:rows.start + rows.size], wd_buf[rows, :], preferred_element_type=f32)
        out = out + (1.0 - gate) * part[0:1]
    o_ref[0] = out.astype(o_ref.dtype)


@jax.jit
def pallas_gated_mix__sliding_block_cached__swiglu_ffn__decode_kernel(
    A_x: jax.Array,
    A_k_cache: jax.Array,
    A_v_cache: jax.Array,
    A_wq: jax.Array,
    A_wo: jax.Array,
    B_x: jax.Array,
    B_w_gate: jax.Array,
    B_w_up: jax.Array,
    B_w_down: jax.Array,
    gate_w: jax.Array,
):
    del B_x
    d_model = A_x.shape[-1]
    ffn = B_w_down.shape[0]
    cache_len = A_k_cache.shape[2]
    window = min(4096, max(256, cache_len // 4))
    assert A_x.shape == (1, 1, d_model) and A_k_cache.shape == (1, _HQ, cache_len, _DH)
    assert window % _CHUNK == 0 and cache_len % _PIECE == 0 and ffn % 32 == 0

    wq = A_wq.reshape(_HQ // _HG, 2, d_model // 8, _HQ * _DH)
    wo = A_wo.reshape(_HQ // _HG, 2, _HG * _DH // 2, d_model)
    wg = B_w_gate.T.reshape(2, ffn // 2, d_model)
    wu = B_w_up.T.reshape(2, ffn // 2, d_model)
    gw = gate_w.reshape(d_model // 128, 128)
    operands = (A_x, A_k_cache, A_v_cache, wq, wo, wg, wu, B_w_down, gw)

    return pl.pallas_call(
        functools.partial(_kernel, window=window),
        out_shape=jax.ShapeDtypeStruct(A_x.shape, A_x.dtype),
        in_specs=[pl.BlockSpec(memory_space=pltpu.HBM)] * len(operands),
        out_specs=pl.BlockSpec(memory_space=pltpu.VMEM),
        scratch_shapes=[
            *(pltpu.VMEM(a.shape, a.dtype) for a in (A_x, gw, wq, wo, wg, wu, B_w_down)),
            pltpu.VMEM((2, _HG, _CHUNK, _DH), A_k_cache.dtype),
            pltpu.VMEM((_NSEM, _HG, _CHUNK, _DH), A_v_cache.dtype),
            pltpu.SemaphoreType.DMA((_NSEM,)),
        ],
        compiler_params=pltpu.CompilerParams(vmem_limit_bytes=48 * 1024 * 1024),
    )(*operands)
```

```python
import functools

import jax
import jax.numpy as jnp
import numpy as np
from jax import lax
import jax.experimental.pallas as pl
import jax.experimental.pallas.tpu as pltpu

_HQ, _DH = 32, 128
_HG = 8
_CHUNK = 512
_PIECE = 64
_PAIRS = _HG // 2
_NSEM = 3
_LAST_STAGE = 96
_NT = (((1,), (1,)), ((), ()))
_F32_MIN = float(np.finfo(np.float32).min)


def _loop(n, body):
    def step(j, carry):
        body(j)
        return carry

    lax.fori_loop(0, n, step, 0)


def _wait_filled(buf, sem):
    pltpu.make_async_copy(buf, buf, sem).wait()


def _row_h_of(vals):
    row = lax.broadcasted_iota(jnp.int32, vals[0].shape, 0)
    out = vals[0]
    for h in range(1, len(vals)):
        out = jnp.where(row == h, vals[h], out)
    return out


def _kernel(x_hbm, k_hbm, v_hbm, wq_hbm, wo_hbm, wg_hbm, wu_hbm, wd_hbm, gw_hbm,
            o_ref,
            x_buf, gw_buf, wq_buf, wo_buf, wg_buf, wu_buf, wd_buf, k_buf, v_buf, sems,
            *, window):
    f32 = jnp.float32
    mxu_dtype = k_buf.dtype
    ffn, d_model = wd_buf.shape
    win_start = k_hbm.shape[2] - window
    n_chunks = window // _CHUNK
    n_groups = _HQ // _HG
    n_steps = n_groups * n_chunks
    n_pieces = _CHUNK // _PIECE
    wd_rows = 2 * _PIECE * _DH // d_model
    wd_first = n_pieces * _PAIRS * wd_rows
    wd_stages = (wd_first, ffn - wd_first - _LAST_STAGE, _LAST_STAGE)

    def sem_of(step):
        return sems.at[lax.rem(step, _NSEM)]

    def cache_copy(src, dst, step, j, t):
        head = lax.div(step, n_chunks) * _HG + 2 * t
        row = pl.multiple_of(j * _PIECE, _PIECE)
        src_row = pl.multiple_of(win_start + lax.rem(step, n_chunks) * _CHUNK + row, _PIECE)
        return pltpu.make_async_copy(
            src.at[0, pl.ds(head, 2), pl.ds(src_row, _PIECE), :],
            dst.at[lax.rem(step, dst.shape[0]), pl.ds(2 * t, 2), pl.ds(row, _PIECE), :],
            sem_of(step))

    k_copy = functools.partial(cache_copy, k_hbm, k_buf)
    v_copy = functools.partial(cache_copy, v_hbm, v_buf)

    def wd_copy(step, j, t):
        rows = pl.ds(pl.multiple_of((j * _PAIRS + t) * wd_rows, wd_rows), wd_rows)
        return pltpu.make_async_copy(wd_hbm.at[rows, :], wd_buf.at[rows, :], sem_of(step))

    def wd_stage(i):
        return pl.ds(sum(wd_stages[:i]), wd_stages[i]), sems.at[(n_steps + i) % _NSEM]

    def start_step(step, ahead_copy):
        def body(j):
            for t in range(_PAIRS):
                k_copy(step, j, t).start(priority=0)
                ahead_copy(step + 1, j, t).start(priority=1)

        _loop(n_pieces, body)

    ffn_sem, proj_sem = sems.at[1], sems.at[2]

    def start_gate_up(j):
        rows = pl.ds(pl.multiple_of(j * 16, 16), 16)
        pltpu.make_async_copy(wg_hbm.at[:, rows, :], wg_buf.at[:, rows, :], ffn_sem).start(priority=0)
        pltpu.make_async_copy(wu_hbm.at[:, rows, :], wu_buf.at[:, rows, :], ffn_sem).start(priority=1)

    _loop(wg_buf.shape[1] // 16, start_gate_up)
    x_copy = pltpu.make_async_copy(x_hbm, x_buf, ffn_sem)
    gw_copy = pltpu.make_async_copy(gw_hbm, gw_buf, ffn_sem)
    x_copy.start()
    gw_copy.start()

    wq_cols = 2 * d_model
    wq_col_blocks = _HQ * _DH // wq_cols

    def start_projections(j):
        q_row = lax.div(j, wq_col_blocks)
        q_cols = pl.ds(pl.multiple_of(lax.rem(j, wq_col_blocks) * wq_cols, wq_cols), wq_cols)
        o_rows = pl.ds(pl.multiple_of(j * 16, 16), 16)
        for t in range(wq_buf.shape[0]):
            pltpu.make_async_copy(wq_hbm.at[t, :, q_row, :, q_cols], wq_buf.at[t, :, q_row, :, q_cols],
                                  proj_sem).start(priority=0)
            pltpu.make_async_copy(wo_hbm.at[t, :, o_rows, :], wo_buf.at[t, :, o_rows, :],
                                  proj_sem).start(priority=1)

    _loop(wo_buf.shape[2] // 16, start_projections)

    x_copy.wait()
    gw_copy.wait()
    _wait_filled(wg_buf, ffn_sem)
    _wait_filled(wu_buf, ffn_sem)
    x = x_buf[0].astype(f32)
    x_rows = jnp.broadcast_to(x, (_HG, d_model)).astype(mxu_dtype)
    gate_w = gw_buf[...].astype(f32)
    lanes = gate_w.shape[1]
    logit = sum(x[:, i * lanes:(i + 1) * lanes] * gate_w[i:i + 1, :] for i in range(gate_w.shape[0]))
    gate = jax.nn.sigmoid(jnp.sum(logit, axis=-1, keepdims=True))
    pre_gate = lax.dot_general(x_rows, wg_buf[...].reshape(ffn, d_model), _NT, preferred_element_type=f32)
    pre_up = lax.dot_general(x_rows, wu_buf[...].reshape(ffn, d_model), _NT, preferred_element_type=f32)
    hidden = (pre_gate * jax.nn.sigmoid(pre_gate) * pre_up).astype(mxu_dtype)

    def start_first_v(j):
        for t in range(_PAIRS):
            v_copy(0, j, t).start(priority=t % 2)

    _loop(n_pieces, start_first_v)
    start_step(0, v_copy)
    _wait_filled(wq_buf, proj_sem)
    _wait_filled(wo_buf, proj_sem)

    def group(g, acc):
        cols = pl.ds(pl.multiple_of(g * (_HG * _DH), _HG * _DH), _HG * _DH)
        q_all = jnp.dot(x_rows, wq_buf[:, :, :, :, cols].reshape(d_model, _HG * _DH), preferred_element_type=f32)
        q = _row_h_of([q_all[:, h * _DH:(h + 1) * _DH] for h in range(_HG)]).astype(mxu_dtype)

        def chunk(c, carry):
            m, l, o = carry
            step = g * n_chunks + c

            @pl.when(step + 2 < n_steps)
            def _():
                start_step(step + 1, v_copy)

            @pl.when(step + 2 == n_steps)
            def _():
                start_step(step + 1, wd_copy)

            k_slot = lax.rem(step, k_buf.shape[0])
            v_slot = lax.rem(step, v_buf.shape[0])
            _wait_filled(k_buf.at[k_slot], sem_of(step))
            _wait_filled(v_buf.at[v_slot], sem_of(step))

            @pl.when(step + 1 == n_steps)
            def _():
                for i in range(1, len(wd_stages)):
                    rows, sem = wd_stage(i)
                    pltpu.make_async_copy(wd_hbm.at[rows, :], wd_buf.at[rows, :], sem).start(priority=1)

            s = _row_h_of([lax.dot_general(q, k_buf[k_slot, h], _NT, preferred_element_type=f32)
                           for h in range(_HG)]) * (_DH ** -0.5)
            m_new = jnp.maximum(m, jnp.max(s, axis=-1, keepdims=True))
            alpha = jnp.exp(m - m_new)
            p = jnp.exp(s - m_new)
            l_new = alpha * l + jnp.sum(p, axis=-1, keepdims=True)
            p = p.astype(mxu_dtype)
            pv = _row_h_of([jnp.dot(p, v_buf[v_slot, h], preferred_element_type=f32) for h in range(_HG)])
            return m_new, l_new, alpha * o + pv

        init = (jnp.full((_HG, 1), _F32_MIN, f32), jnp.zeros((_HG, 1), f32), jnp.zeros((_HG, _DH), f32))
        _, l, o = lax.fori_loop(0, n_chunks, chunk, init)
        o = (o / l).astype(mxu_dtype)
        per_half = _HG // 2
        return acc + _row_h_of([
            jnp.dot(o, wo_buf[g, h // per_half, pl.ds((h % per_half) * _DH, _DH), :], preferred_element_type=f32)
            for h in range(_HG)])

    attn = lax.fori_loop(0, n_groups, group, jnp.zeros((_HG, d_model), f32))

    out = gate * jnp.sum(attn, axis=0, keepdims=True)
    for i in range(len(wd_stages)):
        rows, sem = wd_stage(i)
        _wait_filled(wd_buf.at[rows, :], sem)
        part = jnp.dot(hidden[:, rows.start:rows.start + rows.size], wd_buf[rows, :], preferred_element_type=f32)
        out = out + (1.0 - gate) * part[0:1]
    o_ref[0] = out.astype(o_ref.dtype)


@jax.jit
def pallas_gated_mix__sliding_block_cached__swiglu_ffn__decode_kernel(
    A_x: jax.Array,
    A_k_cache: jax.Array,
    A_v_cache: jax.Array,
    A_wq: jax.Array,
    A_wo: jax.Array,
    B_x: jax.Array,
    B_w_gate: jax.Array,
    B_w_up: jax.Array,
    B_w_down: jax.Array,
    gate_w: jax.Array,
):
    del B_x
    d_model = A_x.shape[-1]
    ffn = B_w_down.shape[0]
    cache_len = A_k_cache.shape[2]
    window = min(4096, max(256, cache_len // 4))
    assert A_x.shape == (1, 1, d_model) and A_k_cache.shape == (1, _HQ, cache_len, _DH)
    assert window % _CHUNK == 0 and cache_len % _PIECE == 0 and ffn % 32 == 0

    wq = A_wq.reshape(_HQ // _HG, 2, d_model // 64, 8, _HQ * _DH)
    wo = A_wo.reshape(_HQ // _HG, 2, _HG * _DH // 2, d_model)
    wg = B_w_gate.T.reshape(2, ffn // 2, d_model)
    wu = B_w_up.T.reshape(2, ffn // 2, d_model)
    gw = gate_w.reshape(d_model // 128, 128)
    operands = (A_x, A_k_cache, A_v_cache, wq, wo, wg, wu, B_w_down, gw)

    return pl.pallas_call(
        functools.partial(_kernel, window=window),
        out_shape=jax.ShapeDtypeStruct(A_x.shape, A_x.dtype),
        in_specs=[pl.BlockSpec(memory_space=pltpu.HBM)] * len(operands),
        out_specs=pl.BlockSpec(memory_space=pltpu.VMEM),
        scratch_shapes=[
            *(pltpu.VMEM(a.shape, a.dtype) for a in (A_x, gw, wq, wo, wg, wu, B_w_down)),
            pltpu.VMEM((2, _HG, _CHUNK, _DH), A_k_cache.dtype),
            pltpu.VMEM((_NSEM, _HG, _CHUNK, _DH), A_v_cache.dtype),
            pltpu.SemaphoreType.DMA((_NSEM,)),
        ],
        compiler_params=pltpu.CompilerParams(vmem_limit_bytes=48 * 1024 * 1024),
    )(*operands)
```
